```python
import os as _os
_os.environ.setdefault("JAX_PLATFORMS", "cpu")
import jax
import jax.numpy as jnp

def _softmax(x, axis=-1):
    return jax.nn.softmax(x, axis=axis)
def _gelu(x):
    return jax.nn.gelu(x, approximate=True)
def _silu(x):
    return jax.nn.silu(x)
def _sigmoid(x):
    return jax.nn.sigmoid(x)
def _layernorm(x, axis=-1, eps=1e-5):
    m = jnp.mean(x, axis=axis, keepdims=True)
    v = jnp.var(x, axis=axis, keepdims=True)
    return (x - m) / jnp.sqrt(v + eps)
def _scatter_add(tgt, idx, src, axis=0):
    return tgt.at[idx].add(src)
def _segment_sum(src, seg, n):
    return jax.ops.segment_sum(src, seg, n)
class _Rng:
    def __init__(self, key):
        self._k = key
    def _next(self):
        self._k, sub = jax.random.split(self._k)
        return sub
    def normal(self, shape):
        return jax.random.normal(self._next(), shape, dtype=jnp.bfloat16)
    def randint(self, lo, hi, shape):
        return jax.random.randint(self._next(), shape, lo, hi, dtype=jnp.int32)
    def uniform(self, shape, lo=0.0, hi=1.0):
        return jax.random.uniform(self._next(), shape, jnp.bfloat16, lo, hi)
    def permutation(self, n):
        return jax.random.permutation(self._next(), n)


kernel_name = 'parallel_sum__sliding_local_dilated__dense_activation_mish__prompt'

def setup_inputs():
    _rng = _Rng(jax.random.key(int.from_bytes(__import__("os").urandom(4), "little")))
    _w = (lambda a: (lambda t: t.astype(jnp.bfloat16) if jnp.issubdtype(t.dtype, jnp.floating) else t)(jnp.asarray(a)))
    def _A_setup():
        B, S, D = 1, 2048, 576
        return {
            "x": _w((lambda *s: _rng.normal(s) * 0.05)(B, S, D)),
            "wqkv": _w((lambda *s: _rng.normal(s) * 0.05)(D, 3 * D)),
            "wo": _w((lambda *s: _rng.normal(s) * 0.05)(D, D)),
        }
    _A_in = _A_setup()

    def _B_setup():
        B, S, D, F = 1, 2048, 576, 4608
        return {
            "x": _w((lambda *s: _rng.normal(s) * 0.05)(B, S, D)),
            "w1": _w((lambda *s: _rng.normal(s) * 1.6)(D, F) * (D ** -0.5)),
            "b1": _w((lambda *s: _rng.normal(s) * 0.2)(F)),
            "w2": _w((lambda *s: _rng.normal(s) * 0.2)(F, D) * (F ** -0.5)),
        }
    _B_in = _B_setup()

    return {
        "A_x": _A_in["x"],
        "A_wqkv": _A_in["wqkv"],
        "A_wo": _A_in["wo"],
        "B_x": _B_in["x"],
        "B_w1": _B_in["w1"],
        "B_b1": _B_in["b1"],
        "B_w2": _B_in["w2"],
    }

def reference(A_x, A_wqkv, A_wo, B_x, B_w1, B_b1, B_w2):
    def _A_ref(x, wqkv, wo):
        B, S, D = x.shape
        H = 32; Dh = D // H
        W, dil = 8, 2
        qkv = (lambda x, *d: x.transpose(*d))((x @ wqkv).reshape(B, S, 3, H, Dh), 2, 0, 3, 1, 4)
        q, k, v = qkv[0], qkv[1], qkv[2]
        scale = Dh ** -0.5
        pos = jnp.arange(S)
        off = jnp.arange(W) * dil
        idx = pos[:, None] - off[None, :]
        mask = idx >= 0
        idx_c = jnp.where(mask, idx, 0).reshape(-1)
        kg = k[:, :, idx_c, :].reshape(B, H, S, W, Dh)
        vg = v[:, :, idx_c, :].reshape(B, H, S, W, Dh)
        logits = jnp.einsum("bhsd,bhswd->bhsw", q, kg) * scale
        logits = jnp.where(mask[None, None, :, :], logits, -1e9)
        attn = _softmax(logits, axis=-1)
        o = jnp.einsum("bhsw,bhswd->bhsd", attn, vg)
        return (lambda x, *d: x.transpose(*d))(o, 0, 2, 1, 3).reshape(B, S, D) @ wo

    def _B_ref(x, w1, b1, w2):
        h = jnp.einsum("bsd,df->bsf", x, w1) + b1
        sp = jnp.log1p(jnp.exp(-jnp.abs(h))) + jnp.where(h > 0, h, jnp.zeros_like(h))
        act = h * jnp.tanh(sp)
        return jnp.einsum("bsf,fd->bsd", act, w2)

    x = A_x
    xn = _layernorm(x, axis=-1)
    return x + _A_ref(xn, A_wqkv, A_wo) + _B_ref(xn, B_w1, B_b1, B_w2)
```

```python
import functools

import jax
import jax.numpy as jnp
import jax.experimental.pallas as pl
import jax.experimental.pallas.tpu as pltpu

S, D, F = 2048, 576, 4608
H, DH, W, DIL = 32, 18, 8, 2
KP = 640
NT = S // 128
NF = F // 128
KT = KP // 128
LOG2E = 1.4426950408889634
LN2 = 0.6931471805599453
LOG2E_HI = 1.4453125
LOG2E_LO = LOG2E - LOG2E_HI
EPS = 1e-5
F32 = jnp.float32
BF16 = jnp.bfloat16
U32 = jnp.uint32


def _dot(a, b):
    return jnp.dot(a, b, preferred_element_type=F32)


def _mish_scaled(hs):
    e = jnp.exp2(jnp.minimum(hs, 30.0))
    n = e * (e + 2.0)
    return (hs * n) * pl.reciprocal(n + 2.0, approx=True)


def make_kernel(A1=2, A2=1, B=4, GT=2, PGROUPS=(1, 1, 2, 4, 8), EGROUPS=(4, 4, 4, 2, 1, 1), scopes=False):
    NL = NT // GT
    A = A1 + A2
    C = NF - A - NL * B
    assert C > 0
    assert A2 >= 0 and sum(PGROUPS) == NT and sum(EGROUPS) == NT

    S_B1, S_WQ, S_WO = 0, 1, 2
    S_X = 3
    S_W1 = S_X + NT
    chunks = [(0, A1)] + ([(A1, A2)] if A2 else []) + [(A + i * B, B) for i in range(NL)] + [(A + NL * B, C)]
    S_W2 = S_W1 + len(chunks)
    S_OUT = S_W2 + NF
    NSEM = S_OUT + NT
    L0 = len(chunks) - NL - 1

    def scope(name):
        import contextlib
        return jax.named_scope(name) if scopes else contextlib.nullcontext()

    def kernel(x_hbm, wqkv_hbm, wo_hbm, w1_hbm, b1_hbm, w2_hbm, out_hbm,
               xs, xn, w1s, w2s, wqs, wqT, wos, woT, b1s, acc, qkv, oT, stg, sems):
        xs_u = xs.bitcast(U32)
        xn_u = xn.bitcast(U32)
        w2_u = w2s.bitcast(U32)

        def x_cp(j):
            return pltpu.make_async_copy(x_hbm.at[:, j * 128:(j + 1) * 128], xs.at[j], sems.at[S_X + j])

        def w1_cp(ci):
            f0, nf = chunks[ci]
            return pltpu.make_async_copy(w1_hbm.at[:, f0 * 128:(f0 + nf) * 128],
                                         w1s.at[0:D, f0 * 128:(f0 + nf) * 128], sems.at[S_W1 + ci])

        def w2_cp(f):
            return pltpu.make_async_copy(w2_hbm.at[:, f * 128:(f + 1) * 128], w2s.at[f], sems.at[S_W2 + f])

        def b1_cp():
            return pltpu.make_async_copy(b1_hbm, b1s, sems.at[S_B1])

        def wq_cp():
            return pltpu.make_async_copy(wqkv_hbm, wqs.at[0:D, :], sems.at[S_WQ])

        def wo_cp():
            return pltpu.make_async_copy(wo_hbm, wos.at[0:D, :], sems.at[S_WO])

        def out_cp(j):
            return pltpu.make_async_copy(stg.at[j], out_hbm.at[:, j * 128:(j + 1) * 128], sems.at[S_OUT + j])

        def start_chunk(ci):
            w1_cp(ci).start()
            f0, nf = chunks[ci]
            for f in range(f0, f0 + nf):
                w2_cp(f).start()

        with scope('ISSUE'):
            b1_cp().start()
            x_cp(0).start()
            w1_cp(0).start()
            x_cp(1).start()
            for f in range(A1):
                w2_cp(f).start()
            for j in range(2, NT):
                x_cp(j).start()
            if A2:
                start_chunk(1)
            wq_cp().start()
            wo_cp().start()
            for ci in range(L0, len(chunks)):
                start_chunk(ci)

        def as_bf16(u):
            return pltpu.bitcast(u, BF16)

        def layernorm_tile(j):
            x = as_bf16(xs_u[j]).astype(F32)
            m = jnp.sum(x, axis=0, keepdims=True) * (1.0 / D)
            xc = x - m
            v = jnp.sum(xc * xc, axis=0, keepdims=True) * (1.0 / D)
            r = jax.lax.rsqrt(v + EPS) * LOG2E
            xn[j, 0:D, :] = (xc * r).astype(BF16)

        def xn_cols(j0, n):
            return jnp.concatenate([as_bf16(xn_u[j0 + t]) for t in range(n)], axis=1)

        def w2_chunk(f0, nf):
            return jnp.concatenate([as_bf16(w2_u[f0 + t]) for t in range(nf)], axis=1)

        def ffn_up(w1T, j0, n):
            return _mish_scaled(_dot(w1T, xn_cols(j0, n))).astype(BF16)

        with scope('PRO'):
            w1s[D + 16:KP, :] = jnp.zeros((KP - D - 16, F), BF16)
            wqs[D:KP, :] = jnp.zeros((KP - D, 3 * D), BF16)
            wos[D:KP, :] = jnp.zeros((KP - D, D), BF16)
            row = jax.lax.broadcasted_iota(jnp.int32, (KP - D, 128), 0)
            ones_rows = jnp.where(row == 0, LOG2E_HI, jnp.where(row == 1, LOG2E_LO, 0.0)).astype(BF16)
            for j in range(NT):
                xn[j, D:KP, :] = ones_rows
            b1_cp().wait()
            b1f = b1s[...].astype(F32)
            row16 = jax.lax.broadcasted_iota(jnp.int32, (16, 128), 0)
            for f in range(NF):
                bb = jnp.broadcast_to(b1f[f:f + 1, :], (16, 128))
                w1s[D:D + 16, f * 128:(f + 1) * 128] = jnp.where(row16 < 2, bb, 0.0).astype(BF16)

            starts = [sum(PGROUPS[:g]) for g in range(len(PGROUPS))]
            for t in range(PGROUPS[0]):
                x_cp(t).wait()
            for t in range(PGROUPS[0]):
                layernorm_tile(t)
            w1_cp(0).wait()
            w1T = w1s[:, 0:A1 * 128].T
            prev = None
            for g in range(len(PGROUPS) + 1):
                if g + 1 < len(PGROUPS):
                    for t in range(PGROUPS[g + 1]):
                        x_cp(starts[g + 1] + t).wait()
                if g == 1:
                    for f in range(A1):
                        w2_cp(f).wait()
                if g == len(PGROUPS):
                    if A2:
                        w1_cp(1).wait()
                        for f in range(A1, A):
                            w2_cp(f).wait()
                cur = ffn_up(w1T, starts[g], PGROUPS[g]) if g < len(PGROUPS) else None
                if g + 1 < len(PGROUPS):
                    for t in range(PGROUPS[g + 1]):
                        layernorm_tile(starts[g + 1] + t)
                if g == len(PGROUPS) and A2:
                    w1Tb = w1s[:, A1 * 128:A * 128].T
                    actb = ffn_up(w1Tb, 0, NT)
                if prev is not None:
                    res = _dot(w2_chunk(0, A1), prev)
                    for t in range(PGROUPS[g - 1]):
                        acc[starts[g - 1] + t] = res[:, t * 128:(t + 1) * 128]
                prev = cur
            wq_cp().wait()
            wo_cp().wait()
            for k in range(KT):
                wqT[k] = pltpu.bitcast(wqs[k * 128:(k + 1) * 128, :].T, U32)
            for k in range(KT):
                woT[k] = pltpu.bitcast(wos[k * 128:(k + 1) * 128, :].T, U32)
            if A2:
                res = _dot(w2_chunk(A1, A2), actb)
                for t in range(NT):
                    acc[t] += res[:, t * 128:(t + 1) * 128]

        lane = jax.lax.broadcasted_iota(jnp.int32, (8, 128), 1)
        qk_scale = (DH ** -0.5) * LN2
        neg = -1e9 * LOG2E

        def shifted(cur, prev, w):
            if w == 0:
                return cur
            dl = DIL * w
            return pltpu.roll(jnp.where(lane >= 128 - dl, prev, cur), dl, 1)

        def attention_tile(j, slot):
            jp = jnp.maximum(j - 1, 0)
            pos = lane + j * 128
            for g in range(H // 8):
                lg = [None] * W
                for d in range(DH):
                    r = 8 * DH * g + d
                    q = qkv[j, pl.ds(r, 8, stride=DH), :]
                    kc = qkv[j, pl.ds(D + r, 8, stride=DH), :]
                    kp = qkv[jp, pl.ds(D + r, 8, stride=DH), :]
                    for w in range(W):
                        t = q * shifted(kc, kp, w)
                        lg[w] = t if d == 0 else lg[w] + t
                lg = [lg[w] * qk_scale for w in range(W)]
                lg = [lg[0]] + [jnp.where(pos >= DIL * w, lg[w], neg) for w in range(1, W)]
                mx = functools.reduce(jnp.maximum, lg)
                p = [jnp.exp2(l - mx) for l in lg]
                rs = pl.reciprocal(functools.reduce(jnp.add, p), approx=True)
                p = [pw * rs for pw in p]
                for d in range(DH):
                    r = 8 * DH * g + d
                    vc = qkv[j, pl.ds(2 * D + r, 8, stride=DH), :]
                    vp = qkv[jp, pl.ds(2 * D + r, 8, stride=DH), :]
                    o = p[0] * vc
                    for w in range(1, W):
                        o = o + p[w] * shifted(vc, vp, w)
                    oT[slot, pl.ds(r, 8, stride=DH), :] = o

        def qkv_group(j0):
            wq_all = jnp.concatenate([as_bf16(wqT[k]) for k in range(KT)], axis=1)
            qkv_g = _dot(wq_all, xn_cols(j0, GT))
            for t in range(GT):
                qkv[j0 + t] = qkv_g[:, t * 128:(t + 1) * 128]

        def wo_group():
            wo_all = jnp.concatenate([as_bf16(woT[k]) for k in range(KT)], axis=1)[:, 0:D]
            o_g = jnp.concatenate([oT[t] for t in range(GT)], axis=1).astype(BF16)
            return _dot(wo_all, o_g)

        def body(i, carry):
            with scope('BODY'):
                f0 = A + i * B
                pltpu.make_async_copy(w1_hbm.at[:, 0:B * 128], w1s.at[0:D, 0:B * 128],
                                      sems.at[S_W1 + L0 + i]).wait()
                for t in range(B):
                    pltpu.make_async_copy(w2_hbm.at[:, 0:128], w2s.at[f0 + t], sems.at[S_W2 + f0 + t]).wait()
                j0 = i * GT
                qkv_group(j0)
                c0 = pl.multiple_of(f0 * 128, 128)
                w1T = w1s[:, pl.ds(c0, B * 128)].T
                act = ffn_up(w1T, 0, NT)
                for t in range(GT):
                    attention_tile(j0 + t, t)
                res = _dot(w2_chunk(f0, B), act)
                for t in range(NT):
                    acc[t] += res[:, t * 128:(t + 1) * 128]
                res2 = wo_group()
                for t in range(GT):
                    acc[j0 + t] += res2[:, t * 128:(t + 1) * 128]
            return carry

        with scope('LOOP'):
            jax.lax.fori_loop(0, NL, body, 0)

        with scope('EPI'):
            f0 = A + NL * B
            w1_cp(len(chunks) - 1).wait()
            for f in range(f0, NF):
                w2_cp(f).wait()
            w1T = w1s[:, f0 * 128:].T
            w2c = w2_chunk(f0, C)
            est = [sum(EGROUPS[:g]) for g in range(len(EGROUPS))]
            nxt = ffn_up(w1T, est[0], EGROUPS[0])
            for g, n in enumerate(EGROUPS):
                act = nxt
                if g + 1 < len(EGROUPS):
                    nxt = ffn_up(w1T, est[g + 1], EGROUPS[g + 1])
                res = _dot(w2c, act)
                for t in range(n):
                    j = est[g] + t
                    y = (acc[j] + res[:, t * 128:(t + 1) * 128]) * LN2 + as_bf16(xs_u[j]).astype(F32)
                    stg[j] = y.astype(BF16)
                    out_cp(j).start()
        with scope('OUTWAIT'):
            for j in range(NT):
                out_cp(j).wait()

    scratch = [
        pltpu.VMEM((NT, D, 128), BF16),
        pltpu.VMEM((NT, KP, 128), BF16),
        pltpu.VMEM((KP, F), BF16),
        pltpu.VMEM((NF, D, 128), BF16),
        pltpu.VMEM((KP, 3 * D), BF16),
        pltpu.VMEM((KT, 3 * D // 2, 128), U32),
        pltpu.VMEM((KP, D), BF16),
        pltpu.VMEM((KT, D // 2, 128), U32),
        pltpu.VMEM((NF, 128), BF16),
        pltpu.VMEM((NT, D, 128), F32),
        pltpu.VMEM((NT, 3 * D, 128), F32),
        pltpu.VMEM((GT, D, 128), F32),
        pltpu.VMEM((NT, D, 128), BF16),
        pltpu.SemaphoreType.DMA((NSEM,)),
    ]

    def fn(A_x, A_wqkv, A_wo, B_x, B_w1, B_b1, B_w2):
        xt = jnp.transpose(A_x[0])
        w2t = jnp.transpose(B_w2)
        b1 = B_b1.reshape(NF, 128)
        out_t = pl.pallas_call(
            kernel,
            in_specs=[pl.BlockSpec(memory_space=pl.ANY)] * 6,
            out_specs=pl.BlockSpec(memory_space=pl.ANY),
            out_shape=jax.ShapeDtypeStruct((D, S), BF16),
            scratch_shapes=scratch,
            compiler_params=pltpu.CompilerParams(vmem_limit_bytes=110 * 1024 * 1024),
            name="fused_block",
        )(xt, A_wqkv, A_wo, B_w1, b1, w2t)
        return jnp.transpose(out_t)[None]

    return fn


_impl = make_kernel()


@jax.jit
def pallas_parallel_sum__sliding_local_dilated__dense_activation_mish__prompt_kernel(
    A_x: jax.Array,
    A_wqkv: jax.Array,
    A_wo: jax.Array,
    B_x: jax.Array,
    B_w1: jax.Array,
    B_b1: jax.Array,
    B_w2: jax.Array,
):
    return _impl(A_x, A_wqkv, A_wo, B_x, B_w1, B_b1, B_w2)
```

```python
import contextlib
import functools

import jax
import jax.numpy as jnp
import jax.experimental.pallas as pl
import jax.experimental.pallas.tpu as pltpu

S, D, F = 2048, 576, 4608
H, DH, W, DIL = 32, 18, 8, 2
KP = 640
NT = S // 128
NF = F // 128
KT = KP // 128
LOG2E = 1.4426950408889634
LN2 = 0.6931471805599453
LOG2E_HI = 1.4453125
LOG2E_LO = LOG2E - LOG2E_HI
EPS = 1e-5
F32 = jnp.float32
BF16 = jnp.bfloat16
U32 = jnp.uint32


def _dot(a, b):
    return jnp.dot(a, b, preferred_element_type=F32)


def _mish_scaled(hs):
    e = jnp.exp2(jnp.minimum(hs, 30.0))
    n = e * (e + 2.0)
    return (hs * n) * pl.reciprocal(n + 2.0, approx=True)


def make_kernel(PGROUPS=(2, 2, 4, 8), NBP=12, EG1=1, EG2=1, FQ=2, FV=2, scopes=False, LOOK=True, RB=True):
    A1, B, GT = 2, 4, 2
    NL = NT // GT
    FB = A1
    FL = A1 + 1
    FE = NF - 1
    assert FL + NL * B == FE and sum(PGROUPS) == NT
    NP = len(PGROUPS)
    pst = [sum(PGROUPS[:g]) for g in range(NP)]

    S_X0 = 0
    S_X = 1
    S_B = S_X + NP
    S_WQ = S_B + 1
    S_L0 = S_WQ + 1
    S_REST = S_L0 + 1
    S_OUT = S_REST + 1
    NSEM = S_OUT + 1

    def x_sem(j):
        return S_X0 if j == 0 else S_X + max(g for g in range(NP) if pst[g] <= j)

    def scope(name):
        return jax.named_scope(name) if scopes else contextlib.nullcontext()

    def kernel(x_hbm, wqkv_hbm, wo_hbm, w1_hbm, b1_hbm, w2_hbm, out_hbm,
               xs, xn, w1s, w2s, wqs, wqT, wos, woT, b1s, acc, qkv, stg, sems):
        xn_u = xn
        if RB:
            xs_u = xs.bitcast(U32)
            w2_u = w2s.bitcast(U32)

        def x_cp(j):
            return pltpu.make_async_copy(x_hbm.at[:, j * 128:(j + 1) * 128], xs.at[j], sems.at[x_sem(j)])

        def w1_cp(f0, nf, sem):
            cols = pl.ds(f0 * 128, nf * 128)
            return pltpu.make_async_copy(w1_hbm.at[:, cols], w1s.at[0:D, cols], sems.at[sem])

        def w2_cp(f, sem):
            return pltpu.make_async_copy(w2_hbm.at[:, pl.ds(f * 128, 128)], w2s.at[f], sems.at[sem])

        def chunk_cps(f0, nf, sem):
            return [w1_cp(f0, nf, sem)] + [w2_cp(f, sem) for f in range(f0, f0 + nf)]

        def b1_cp():
            return pltpu.make_async_copy(b1_hbm, b1s, sems.at[S_X0])

        def wq_cps():
            return [pltpu.make_async_copy(wqkv_hbm, wqs.at[0:D, :], sems.at[S_WQ]),
                    pltpu.make_async_copy(wo_hbm, wos.at[0:D, :], sems.at[S_WQ])]

        def rest_cps():
            return chunk_cps(FL + B, NF - FL - B, S_REST)

        def out_cp(j):
            return pltpu.make_async_copy(stg.at[j], out_hbm.at[:, j * 128:(j + 1) * 128], sems.at[S_OUT])

        with scope('ISSUE'):
            b1_cp().start()
            x_cp(0).start()
            w1_cp(0, A1, S_X).start()
            for j in range(1, PGROUPS[0]):
                x_cp(j).start()
            for f in range(A1):
                w2_cp(f, S_X + 1).start()
            for j in range(PGROUPS[0], NT):
                x_cp(j).start()
            for cp in chunk_cps(FB, 1, S_B) + wq_cps() + chunk_cps(FL, B, S_L0) + rest_cps():
                cp.start()

        def as_bf16(u):
            return pltpu.bitcast(u, BF16)

        def pack2(a, b):
            return pltpu.pack_elementwise([a, b], packed_dtype=BF16)

        def unpack2(p):
            return [pltpu.unpack_elementwise(p, index=i, packed_dtype=BF16, unpacked_dtype=F32) for i in range(2)]

        def layernorm_tile(j):
            xe, xo = unpack2(xs_u[j] if RB else pltpu.bitcast(xs[j], U32))
            m = jnp.sum(xe + xo, axis=0, keepdims=True) * (1.0 / D)
            ce, co = xe - m, xo - m
            v = jnp.sum(ce * ce + co * co, axis=0, keepdims=True) * (1.0 / D)
            r = jax.lax.rsqrt(v + EPS) * LOG2E
            xn_u[j, 0:D // 2, :] = pack2(ce * r, co * r).astype(U32)

        def xn_cols(j0, n):
            return jnp.concatenate([as_bf16(xn_u[j0 + t]) for t in range(n)], axis=1)

        def w2_tiles(fs):
            return jnp.concatenate([as_bf16(w2_u[f]) if RB else w2s[f] for f in fs], axis=1)

        def ffn_up(w1T, j0, n):
            return _mish_scaled(_dot(w1T, xn_cols(j0, n))).astype(BF16)

        with scope('PRO'):
            w1s[D + 16:KP, :] = jnp.zeros((KP - D - 16, F), BF16)
            wqs[D:KP, :] = jnp.zeros((KP - D, 3 * D), BF16)
            wos[D:KP, :] = jnp.zeros((KP - D, D), BF16)
            row = jax.lax.broadcasted_iota(jnp.int32, ((KP - D) // 2, 128), 0)
            ones_rows = pack2(jnp.where(row == 0, LOG2E_HI, 0.0), jnp.where(row == 0, LOG2E_LO, 0.0)).astype(U32)
            for j in range(NT):
                xn[j, D // 2:KP // 2, :] = ones_rows
            with scope('W0'):
                b1_cp().wait()
                x_cp(0).wait()
            b1f = b1s[...].astype(F32)
            row16 = jax.lax.broadcasted_iota(jnp.int32, (16, 128), 0)
            for f in range(NF):
                bb = jnp.broadcast_to(b1f[f:f + 1, :], (16, 128))
                w1s[D:D + 16, f * 128:(f + 1) * 128] = jnp.where(row16 < 2, bb, 0.0).astype(BF16)
            layernorm_tile(0)

            def down0(g, act, part):
                r0, r1 = (0, D // 2) if part == 0 else (D // 2, D)
                res = _dot(w2_tiles(range(A1))[r0:r1, :], act)
                for t in range(PGROUPS[g]):
                    acc[pst[g] + t, r0:r1, :] = res[:, t * 128:(t + 1) * 128]

            prev = None
            for g in range(NP):
                tiles = [j for j in range(pst[g], pst[g] + PGROUPS[g]) if j >= 1]
                with scope('WG%d' % g):
                    if g == 0:
                        w1_cp(0, A1, S_X).wait()
                    if g == 1:
                        for f in range(A1):
                            w2_cp(f, S_X + 1).wait()
                    for j in tiles:
                        x_cp(j).wait()
                if g == 0:
                    w1T = w1s[:, 0:A1 * 128].T
                if prev is not None:
                    down0(g - 1, prev, 0)
                for j in tiles:
                    layernorm_tile(j)
                cur = ffn_up(w1T, pst[g], PGROUPS[g])
                if prev is not None:
                    down0(g - 1, prev, 1)
                prev = cur
            with scope('WB'):
                for cp in chunk_cps(FB, 1, S_B):
                    cp.wait()
            w1Tb = w1s[:, FB * 128:(FB + 1) * 128].T
            if NBP == NT:
                down0(NP - 1, prev, 0)
                actb = ffn_up(w1Tb, 0, NBP)
                down0(NP - 1, prev, 1)
            else:
                actb = ffn_up(w1Tb, 0, NBP)
                down0(NP - 1, prev, 0)
            with scope('WQ'):
                for cp in wq_cps():
                    cp.wait()
            if NBP != NT:
                down0(NP - 1, prev, 1)
            for k in range(KT):
                wqT[k] = pltpu.bitcast(wqs[k * 128:(k + 1) * 128, :].T, U32)
            for k in range(KT):
                woT[k] = pltpu.bitcast(wos[k * 128:(k + 1) * 128, :].T, U32)
            res = _dot(w2_tiles([FB]), actb)
            for t in range(NBP):
                acc[t] += res[:, t * 128:(t + 1) * 128]

        lane = jax.lax.broadcasted_iota(jnp.int32, (8, 128), 1)
        qk_scale = (DH ** -0.5) * LN2
        neg = -1e9 * LOG2E

        def shifted(cur, prev, w):
            dl = DIL * w
            return pltpu.roll(jnp.where(lane >= 128 - dl, prev, cur), dl, 1)

        def windows(base, j, jp, r):
            cur = [qkv[j, pl.ds(base + r + u, 8, stride=DH), :] for u in range(2)]
            prv = [qkv[jp, pl.ds(base + r + u, 8, stride=DH), :] for u in range(2)]
            yield 0, cur
            for w in range(1, W):
                yield w, [shifted(cur[u], prv[u], w) for u in range(2)]

        def attention_tile(j):
            jp = jnp.maximum(j - 1, 0)
            pos = lane + j * 128
            for g in range(H // 8):
                lg = [None] * W
                for d in range(0, DH, 2):
                    r = 8 * DH * g + d
                    q = [qkv[j, pl.ds(r + u, 8, stride=DH), :] for u in range(2)]
                    for w, ks in windows(D, j, jp, r):
                        t = q[0] * ks[0] + q[1] * ks[1]
                        lg[w] = t if d == 0 else lg[w] + t
                    if (d // 2) % FQ == FQ - 1:
                        qkv[NT, 0:8, :] = lg[W - 1]
                lg = [lg[w] * qk_scale for w in range(W)]
                lg = [lg[0]] + [jnp.where(pos >= DIL * w, lg[w], neg) for w in range(1, W)]
                mx = functools.reduce(jnp.maximum, lg)
                p = [jnp.exp2(l - mx) for l in lg]
                rs = pl.reciprocal(functools.reduce(jnp.add, p), approx=True)
                p = [pw * rs for pw in p]
                pend = []
                for d in range(0, DH, 2):
                    r = 8 * DH * g + d
                    o = None
                    for w, vs in windows(2 * D, j, jp, r):
                        t = [p[w] * vs[u] for u in range(2)]
                        o = t if o is None else [o[u] + t[u] for u in range(2)]
                    pend += [(r + u, o[u]) for u in range(2)]
                    if (d // 2) % FV == FV - 1 or d == DH - 2:
                        for rr, oo in pend:
                            qkv[j, pl.ds(rr, 8, stride=DH), :] = oo
                        pend = []

        def body(i, carry):
            @pl.when(i == 1)
            def _():
                for cp in rest_cps():
                    cp.wait()

            with scope('BODY'):
                f0 = FL + i * B
                c0 = pl.multiple_of(f0 * 128, 128)
                j0 = i * GT
                wq_all = jnp.concatenate([as_bf16(wqT[k]) for k in range(KT)], axis=1)
                qkv_g = _dot(wq_all, xn_cols(j0, GT))
                for t in range(GT):
                    qkv[j0 + t] = qkv_g[:, t * 128:(t + 1) * 128]
                w1T = w1s[:, pl.ds(c0, B * 128)].T
                act = ffn_up(w1T, 0, NT)
                for t in range(GT):
                    attention_tile(j0 + t)
                res = _dot(w2_tiles([f0 + t for t in range(B)]), act)
                for t in range(NT):
                    acc[t] += res[:, t * 128:(t + 1) * 128]
                wo_all = jnp.concatenate([as_bf16(woT[k]) for k in range(KT)], axis=1)[:, 0:D]
                o_g = jnp.concatenate([qkv[j0 + t, 0:D, :] for t in range(GT)], axis=1).astype(BF16)
                res2 = _dot(wo_all, o_g)
                for t in range(GT):
                    acc[j0 + t] += res2[:, t * 128:(t + 1) * 128]
            return carry

        with scope('LOOP'):
            for cp in chunk_cps(FL, B, S_L0):
                cp.wait()
            jax.lax.fori_loop(0, NL, body, 0)

        with scope('EPI'):
            w1Te = w1s[:, FE * 128:].T
            w2e = w2_tiles([FE])
            groups = [(j, EG1, w1Te, w2e) for j in range(0, NBP, EG1)]
            if NBP < NT:
                w1Tb = w1s[:, FB * 128:(FB + 1) * 128].T
                w1T2 = jnp.concatenate([w1Tb, w1Te], axis=0)
                w2e2 = w2_tiles([FB, FE])
                groups += [(j, EG2, w1T2, w2e2) for j in range(NBP, NT, EG2)]
            nxt = ffn_up(groups[0][2], groups[0][0], groups[0][1])
            for g, (j0, n, _, w2c) in enumerate(groups):
                act = nxt if LOOK or g == 0 else ffn_up(groups[g][2], j0, n)
                if g + 1 < len(groups) and LOOK:
                    nxt = ffn_up(groups[g + 1][2], groups[g + 1][0], groups[g + 1][1])
                res = _dot(w2c, act)
                for t in range(n):
                    j = j0 + t
                    y = (acc[j] + res[:, t * 128:(t + 1) * 128]) * LN2 + (as_bf16(xs_u[j]) if RB else xs[j]).astype(F32)
                    stg[j] = y.astype(BF16)
                    out_cp(j).start()
        with scope('OUTWAIT'):
            for j in range(NT):
                out_cp(j).wait()

    scratch = [
        pltpu.VMEM((NT, D, 128), BF16),
        pltpu.VMEM((NT, KP // 2, 128), U32),
        pltpu.VMEM((KP, F), BF16),
        pltpu.VMEM((NF, D, 128), BF16),
        pltpu.VMEM((KP, 3 * D), BF16),
        pltpu.VMEM((KT, 3 * D // 2, 128), U32),
        pltpu.VMEM((KP, D), BF16),
        pltpu.VMEM((KT, D // 2, 128), U32),
        pltpu.VMEM((NF, 128), BF16),
        pltpu.VMEM((NT, D, 128), F32),
        pltpu.VMEM((NT + 1, 3 * D, 128), F32),
        pltpu.VMEM((NT, D, 128), BF16),
        pltpu.SemaphoreType.DMA((NSEM,)),
    ]

    def fn(A_x, A_wqkv, A_wo, B_x, B_w1, B_b1, B_w2):
        xt = jnp.transpose(A_x[0])
        w2t = jnp.transpose(B_w2)
        b1 = B_b1.reshape(NF, 128)
        out_t = pl.pallas_call(
            kernel,
            in_specs=[pl.BlockSpec(memory_space=pl.ANY)] * 6,
            out_specs=pl.BlockSpec(memory_space=pl.ANY),
            out_shape=jax.ShapeDtypeStruct((D, S), BF16),
            scratch_shapes=scratch,
            compiler_params=pltpu.CompilerParams(vmem_limit_bytes=110 * 1024 * 1024),
            name="fused_block",
        )(xt, A_wqkv, A_wo, B_w1, b1, w2t)
        return jnp.transpose(out_t)[None]

    return fn


_impl = make_kernel(RB=False)


@jax.jit
def pallas_parallel_sum__sliding_local_dilated__dense_activation_mish__prompt_kernel(
    A_x: jax.Array,
    A_wqkv: jax.Array,
    A_wo: jax.Array,
    B_x: jax.Array,
    B_w1: jax.Array,
    B_b1: jax.Array,
    B_w2: jax.Array,
):
    return _impl(A_x, A_wqkv, A_wo, B_x, B_w1, B_b1, B_w2)
```

```python
import functools

import jax
import jax.numpy as jnp
import jax.experimental.pallas as pl
import jax.experimental.pallas.tpu as pltpu

S, D, F = 2048, 576, 4608
H, DH, W, DIL = 32, 18, 8, 2
KP = 640
NT = S // 128
NF = F // 128
KT = KP // 128
LOG2E = 1.4426950408889634
LN2 = 0.6931471805599453
LOG2E_HI = 1.4453125
LOG2E_LO = LOG2E - LOG2E_HI
EPS = 1e-5
F32 = jnp.float32
BF16 = jnp.bfloat16
U32 = jnp.uint32

A1 = 2
FB = A1
FL = A1 + 1
FE = NF - 1
B = 4
GT = 2
NL = NT // GT
NBP = 12
EPRE = 2
PGROUPS = (2, 2, 4, 8)
NP = len(PGROUPS)
PST = [sum(PGROUPS[:g]) for g in range(NP)]
RBS = (144, 288)
FQ = 2
FV = 2
assert FL + NL * B == FE and sum(PGROUPS) == NT

S_X0 = 0
S_X = 1
S_B = S_X + NP
S_WQ = S_B + 1
S_L0 = S_WQ + 1
S_REST = S_L0 + 1
S_OUT = S_REST + 1
NSEM = S_OUT + 1


def _x_sem(j):
    return S_X0 if j == 0 else S_X + max(g for g in range(NP) if PST[g] <= j)


def _dot(a, b):
    return jnp.dot(a, b, preferred_element_type=F32)


def _as_bf16(u):
    return pltpu.bitcast(u, BF16)


def _mish_scaled(hs):
    e = jnp.exp2(jnp.minimum(hs, 13.0))
    n = e * (e + 2.0)
    return (hs * n) * pl.reciprocal(n + 2.0, approx=True)


def _kernel(x_hbm, wqkv_hbm, wo_hbm, w1_hbm, b1_hbm, w2_hbm, out_hbm,
            xs, xn, w1s, w2s, wqs, wqT, wos, woT, b1s, acc, qkv, stg, w1Tbs, sems):

    def x_cp(j):
        return pltpu.make_async_copy(x_hbm.at[:, j * 128:(j + 1) * 128], xs.at[j], sems.at[_x_sem(j)])

    def w1_cp(f0, nf, sem):
        cols = pl.ds(f0 * 128, nf * 128)
        return pltpu.make_async_copy(w1_hbm.at[:, cols], w1s.at[0:D, cols], sems.at[sem])

    def w2_cp(f, sem):
        return pltpu.make_async_copy(w2_hbm.at[:, pl.ds(f * 128, 128)], w2s.at[f], sems.at[sem])

    def chunk_cps(f0, nf, sem):
        return [w1_cp(f0, nf, sem)] + [w2_cp(f, sem) for f in range(f0, f0 + nf)]

    def b1_cp():
        return pltpu.make_async_copy(b1_hbm, b1s, sems.at[S_X0])

    def wq_cps():
        return [pltpu.make_async_copy(wqkv_hbm, wqs.at[0:D, :], sems.at[S_WQ]),
                pltpu.make_async_copy(wo_hbm, wos.at[0:D, :], sems.at[S_WQ])]

    def rest_cps():
        return chunk_cps(FL + B, NF - FL - B, S_REST)

    def out_cp(j, r0, r1):
        return pltpu.make_async_copy(stg.at[j, r0:r1, :], out_hbm.at[r0:r1, j * 128:(j + 1) * 128],
                                     sems.at[S_OUT])

    def out_parts(j):
        return [(0, D // 2), (D // 2, D)] if j == NT - 1 else [(0, D)]

    b1_cp().start()
    x_cp(0).start()
    w1_cp(0, A1, S_X).start()
    for j in range(1, PGROUPS[0]):
        x_cp(j).start()
    for f in range(A1):
        w2_cp(f, S_X + 1).start()
    for j in range(PGROUPS[0], NT):
        x_cp(j).start()
    for cp in chunk_cps(FB, 1, S_B) + wq_cps() + chunk_cps(FL, B, S_L0) + rest_cps():
        cp.start()

    def layernorm_tile(j):
        x = xs[j].astype(F32)
        m = jnp.sum(x, axis=0, keepdims=True) * (1.0 / D)
        xc = x - m
        v = jnp.sum(xc * xc, axis=0, keepdims=True) * (1.0 / D)
        r = jax.lax.rsqrt(v + EPS) * LOG2E
        xn[j, 0:D, :] = (xc * r).astype(BF16)

    def xn_cols(j0, n):
        return jnp.concatenate([_as_bf16(xn.bitcast(U32)[j0 + t]) for t in range(n)], axis=1)

    def w2_tiles(fs):
        return jnp.concatenate([w2s[f] for f in fs], axis=1)

    def ffn_up(w1T, j0, n):
        return _mish_scaled(_dot(w1T, xn_cols(j0, n))).astype(BF16)

    w1s[D + 16:KP, :] = jnp.zeros((KP - D - 16, F), BF16)
    wqs[D:KP, :] = jnp.zeros((KP - D, 3 * D), BF16)
    wos[D:KP, :] = jnp.zeros((KP - D, D), BF16)
    row = jax.lax.broadcasted_iota(jnp.int32, (KP - D, 128), 0)
    ones_rows = jnp.where(row == 0, LOG2E_HI, jnp.where(row == 1, LOG2E_LO, 0.0)).astype(BF16)
    for j in range(NT):
        xn[j, D:KP, :] = ones_rows
    b1_cp().wait()
    x_cp(0).wait()
    b1f = b1s[...].astype(F32)
    row16 = jax.lax.broadcasted_iota(jnp.int32, (16, 128), 0)
    for f in range(NF):
        bb = jnp.broadcast_to(b1f[f:f + 1, :], (16, 128))
        w1s[D:D + 16, f * 128:(f + 1) * 128] = jnp.where(row16 < 2, bb, 0.0).astype(BF16)
    layernorm_tile(0)

    def down0(g, act, r0, r1):
        res = _dot(w2_tiles(range(A1))[r0:r1, :], act)
        for t in range(PGROUPS[g]):
            acc[PST[g] + t, r0:r1, :] = res[:, t * 128:(t + 1) * 128]

    prev = None
    for g in range(NP):
        tiles = [j for j in range(PST[g], PST[g] + PGROUPS[g]) if j >= 1]
        if g == 0:
            w1_cp(0, A1, S_X).wait()
        if g == 1:
            for f in range(A1):
                w2_cp(f, S_X + 1).wait()
        for j in tiles:
            x_cp(j).wait()
        if g == 0:
            w1T = w1s[:, 0:A1 * 128].T
        if prev is not None:
            down0(g - 1, prev, 0, D // 2)
        for j in tiles:
            layernorm_tile(j)
        cur = ffn_up(w1T, PST[g], PGROUPS[g])
        if prev is not None:
            down0(g - 1, prev, D // 2, D)
        prev = cur
    for cp in chunk_cps(FB, 1, S_B):
        cp.wait()
    w1Tb = w1s[:, FB * 128:(FB + 1) * 128].T
    for k in range(KT):
        w1Tbs[k] = pltpu.bitcast(w1Tb[:, k * 128:(k + 1) * 128], U32)
    down0(NP - 1, prev, 0, RBS[0])
    actb = ffn_up(w1Tb, 0, NBP)
    down0(NP - 1, prev, RBS[0], RBS[1])
    for cp in wq_cps():
        cp.wait()
    down0(NP - 1, prev, RBS[1], D)
    for k in range(KT):
        wqT[k] = pltpu.bitcast(wqs[k * 128:(k + 1) * 128, :].T, U32)
    for k in range(KT):
        woT[k] = pltpu.bitcast(wos[k * 128:(k + 1) * 128, :].T, U32)
    res = _dot(w2_tiles([FB]), actb)
    for t in range(NBP):
        acc[t] += res[:, t * 128:(t + 1) * 128]

    lane = jax.lax.broadcasted_iota(jnp.int32, (8, 128), 1)
    qk_scale = (DH ** -0.5) * LN2
    neg = -1e9 * LOG2E

    def windows(base, j, jp, r):
        cur = [qkv[j, pl.ds(base + r + u, 8, stride=DH), :] for u in range(2)]
        prv = [qkv[jp, pl.ds(base + r + u, 8, stride=DH), :] for u in range(2)]
        yield 0, cur
        for w in range(1, W):
            dl = DIL * w
            yield w, [pltpu.roll(jnp.where(lane >= 128 - dl, prv[u], cur[u]), dl, 1) for u in range(2)]

    def attention_tile(j):
        jp = jnp.maximum(j - 1, 0)
        pos = lane + j * 128
        for g in range(H // 8):
            lg = [None] * W
            for d in range(0, DH, 2):
                r = 8 * DH * g + d
                q = [qkv[j, pl.ds(r + u, 8, stride=DH), :] for u in range(2)]
                for w, ks in windows(D, j, jp, r):
                    t = q[0] * ks[0] + q[1] * ks[1]
                    lg[w] = t if d == 0 else lg[w] + t
                if (d // 2) % FQ == FQ - 1:
                    qkv[NT, 0:8, :] = lg[W - 1]
            lg = [lg[w] * qk_scale for w in range(W)]
            lg = [lg[0]] + [jnp.where(pos >= DIL * w, lg[w], neg) for w in range(1, W)]
            mx = functools.reduce(jnp.maximum, lg)
            p = [jnp.exp2(l - mx) for l in lg]
            rs = pl.reciprocal(functools.reduce(jnp.add, p), approx=True)
            p = [pw * rs for pw in p]
            pend = []
            for d in range(0, DH, 2):
                r = 8 * DH * g + d
                o = None
                for w, vs in windows(2 * D, j, jp, r):
                    t = [p[w] * vs[u] for u in range(2)]
                    o = t if o is None else [o[u] + t[u] for u in range(2)]
                pend += [(r + u, o[u]) for u in range(2)]
                if (d // 2) % FV == FV - 1 or d == DH - 2:
                    for rr, oo in pend:
                        qkv[j, pl.ds(rr, 8, stride=DH), :] = oo
                    pend = []

    def body(i, carry):
        @pl.when(i == 1)
        def _():
            for cp in rest_cps():
                cp.wait()

        f0 = FL + i * B
        c0 = pl.multiple_of(f0 * 128, 128)
        j0 = i * GT
        wq_all = jnp.concatenate([_as_bf16(wqT[k]) for k in range(KT)], axis=1)
        qkv_g = _dot(wq_all, xn_cols(j0, GT))
        for t in range(GT):
            qkv[j0 + t] = qkv_g[:, t * 128:(t + 1) * 128]
        w1T = w1s[:, pl.ds(c0, B * 128)].T
        act = ffn_up(w1T, 0, NT)
        for t in range(GT):
            attention_tile(j0 + t)
        res = _dot(w2_tiles([f0 + t for t in range(B)]), act)
        for t in range(NT):
            acc[t] += res[:, t * 128:(t + 1) * 128]
        wo_all = jnp.concatenate([_as_bf16(woT[k]) for k in range(KT)], axis=1)[:, 0:D]
        o_g = jnp.concatenate([qkv[j0 + t, 0:D, :] for t in range(GT)], axis=1).astype(BF16)
        res2 = _dot(wo_all, o_g)
        for t in range(GT):
            acc[j0 + t] += res2[:, t * 128:(t + 1) * 128]
        return carry

    for cp in chunk_cps(FL, B, S_L0):
        cp.wait()
    jax.lax.fori_loop(0, NL, body, 0)

    w1Te = w1s[:, FE * 128:].T
    w2e = w2_tiles([FE])
    w1Tb = jnp.concatenate([_as_bf16(w1Tbs[k]) for k in range(KT)], axis=1)
    w2e2 = w2_tiles([FB, FE])
    pre = {j: ffn_up(w1Tb, j, 1) for j in range(NBP, NBP + EPRE)}

    def up_e(j):
        a = ffn_up(w1Te, j, 1)
        if j >= NBP:
            ab = pre[j] if j in pre else ffn_up(w1Tb, j, 1)
            a = jnp.concatenate([ab, a], axis=0)
        return a

    nxt = up_e(0)
    for j in range(NT):
        act = nxt
        if j + 1 < NT:
            nxt = up_e(j + 1)
        w2c = w2e2 if j >= NBP else w2e
        for r0, r1 in out_parts(j):
            res = _dot(w2c[r0:r1, :], act)
            y = (acc[j, r0:r1, :] + res) * LN2 + xs[j, r0:r1, :].astype(F32)
            stg[j, r0:r1, :] = y.astype(BF16)
            out_cp(j, r0, r1).start()
    for j in range(NT):
        for r0, r1 in out_parts(j):
            out_cp(j, r0, r1).wait()


_SCRATCH = [
    pltpu.VMEM((NT, D, 128), BF16),
    pltpu.VMEM((NT, KP, 128), BF16),
    pltpu.VMEM((KP, F), BF16),
    pltpu.VMEM((NF, D, 128), BF16),
    pltpu.VMEM((KP, 3 * D), BF16),
    pltpu.VMEM((KT, 3 * D // 2, 128), U32),
    pltpu.VMEM((KP, D), BF16),
    pltpu.VMEM((KT, D // 2, 128), U32),
    pltpu.VMEM((NF, 128), BF16),
    pltpu.VMEM((NT, D, 128), F32),
    pltpu.VMEM((NT + 1, 3 * D, 128), F32),
    pltpu.VMEM((NT, D, 128), BF16),
    pltpu.VMEM((KT, 64, 128), U32),
    pltpu.SemaphoreType.DMA((NSEM,)),
]


@jax.jit
def pallas_parallel_sum__sliding_local_dilated__dense_activation_mish__prompt_kernel(
    A_x: jax.Array,
    A_wqkv: jax.Array,
    A_wo: jax.Array,
    B_x: jax.Array,
    B_w1: jax.Array,
    B_b1: jax.Array,
    B_w2: jax.Array,
):
    del B_x
    xt = jnp.transpose(A_x[0])
    w2t = jnp.transpose(B_w2)
    b1 = B_b1.reshape(NF, 128)
    out_t = pl.pallas_call(
        _kernel,
        in_specs=[pl.BlockSpec(memory_space=pl.ANY)] * 6,
        out_specs=pl.BlockSpec(memory_space=pl.ANY),
        out_shape=jax.ShapeDtypeStruct((D, S), BF16),
        scratch_shapes=_SCRATCH,
        compiler_params=pltpu.CompilerParams(vmem_limit_bytes=110 * 1024 * 1024),
        name="fused_block",
    )(xt, A_wqkv, A_wo, B_w1, b1, w2t)
    return jnp.transpose(out_t)[None]
```

```python
import functools

import jax
import jax.numpy as jnp
import jax.experimental.pallas as pl
import jax.experimental.pallas.tpu as pltpu

S, D, F = 2048, 576, 4608
H, DH, W, DIL = 32, 18, 8, 2
KP = 640
NT = S // 128
NF = F // 128
KT = KP // 128
LOG2E = 1.4426950408889634
LN2 = 0.6931471805599453
LOG2E_HI = 1.4453125
LOG2E_LO = LOG2E - LOG2E_HI
EPS = 1e-5
F32 = jnp.float32
BF16 = jnp.bfloat16
U32 = jnp.uint32

A1 = 2
FB = A1
FL = A1 + 1
FE = NF - 1
B = 4
GT = 2
NL = NT // GT
NBP = 12
EPRE = 2
PGROUPS = (2, 2, 4, 8)
NP = len(PGROUPS)
PST = [sum(PGROUPS[:g]) for g in range(NP)]
DS = (432, 432, 480)
RBS = (144, 288)
FQ = 2
FV = 2
assert FL + NL * B == FE and sum(PGROUPS) == NT

S_X0 = 0
S_X = 1
S_B = S_X + NP
S_WQ = S_B + 1
S_L0 = S_WQ + 1
S_REST = S_L0 + 1
S_OUT = S_REST + 1
NSEM = S_OUT + 1


def _x_sem(j):
    return S_X0 if j == 0 else S_X + max(g for g in range(NP) if PST[g] <= j)


def _dot(a, b):
    return jnp.dot(a, b, preferred_element_type=F32)


def _as_bf16(u):
    return pltpu.bitcast(u, BF16)


def _mish_scaled(hs):
    e = jnp.exp2(jnp.minimum(hs, 13.0))
    n = e * (e + 2.0)
    return (hs * n) * pl.reciprocal(n + 2.0, approx=True)


def _kernel(x_hbm, wqkv_hbm, wo_hbm, w1_hbm, b1_hbm, w2_hbm, out_hbm,
            xs, xn, w1s, w2s, wqs, wqT, wos, woT, b1s, acc, qkv, stg, w1Tbs, sems):

    def x_cp(j):
        return pltpu.make_async_copy(x_hbm.at[:, j * 128:(j + 1) * 128], xs.at[j], sems.at[_x_sem(j)])

    def w1_cp(f0, nf, sem):
        cols = pl.ds(f0 * 128, nf * 128)
        return pltpu.make_async_copy(w1_hbm.at[:, cols], w1s.at[0:D, cols], sems.at[sem])

    def w2_cp(f, sem):
        return pltpu.make_async_copy(w2_hbm.at[:, pl.ds(f * 128, 128)], w2s.at[f], sems.at[sem])

    def chunk_cps(f0, nf, sem):
        return [w1_cp(f0, nf, sem)] + [w2_cp(f, sem) for f in range(f0, f0 + nf)]

    def b1_cp():
        return pltpu.make_async_copy(b1_hbm, b1s, sems.at[S_X0])

    def wq_cps():
        return [pltpu.make_async_copy(wqkv_hbm, wqs.at[0:D, :], sems.at[S_WQ]),
                pltpu.make_async_copy(wo_hbm, wos.at[0:D, :], sems.at[S_WQ])]

    def rest_cps():
        return chunk_cps(FL + B, NF - FL - B, S_REST)

    def out_cp(j, r0, r1):
        return pltpu.make_async_copy(stg.at[j, r0:r1, :], out_hbm.at[r0:r1, j * 128:(j + 1) * 128],
                                     sems.at[S_OUT])

    def out_parts(j):
        return [(0, D // 2), (D // 2, D)] if j == NT - 1 else [(0, D)]

    b1_cp().start()
    x_cp(0).start()
    w1_cp(0, A1, S_X).start()
    for j in range(1, PGROUPS[0]):
        x_cp(j).start()
    for f in range(A1):
        w2_cp(f, S_X + 1).start()
    for j in range(PGROUPS[0], NT):
        x_cp(j).start()
    for cp in chunk_cps(FB, 1, S_B) + wq_cps() + chunk_cps(FL, B, S_L0) + rest_cps():
        cp.start()

    def layernorm_tile(j):
        x = xs[j].astype(F32)
        m = jnp.sum(x, axis=0, keepdims=True) * (1.0 / D)
        xc = x - m
        v = jnp.sum(xc * xc, axis=0, keepdims=True) * (1.0 / D)
        r = jax.lax.rsqrt(v + EPS) * LOG2E
        xn[j, 0:D, :] = (xc * r).astype(BF16)

    def xn_cols(j0, n):
        return jnp.concatenate([xn[j0 + t] for t in range(n)], axis=1)

    def w2_tiles(fs):
        return jnp.concatenate([w2s[f] for f in fs], axis=1)

    def ffn_up(w1T, j0, n):
        return _mish_scaled(_dot(w1T, xn_cols(j0, n))).astype(BF16)

    w1s[D + 16:KP, :] = jnp.zeros((KP - D - 16, F), BF16)
    wqs[D:KP, :] = jnp.zeros((KP - D, 3 * D), BF16)
    wos[D:KP, :] = jnp.zeros((KP - D, D), BF16)
    row = jax.lax.broadcasted_iota(jnp.int32, (KP - D, 128), 0)
    ones_rows = jnp.where(row == 0, LOG2E_HI, jnp.where(row == 1, LOG2E_LO, 0.0)).astype(BF16)
    for j in range(NT):
        xn[j, D:KP, :] = ones_rows
    b1_cp().wait()
    x_cp(0).wait()
    b1f = b1s[...].astype(F32)
    row16 = jax.lax.broadcasted_iota(jnp.int32, (16, 128), 0)
    for f in range(NF):
        bb = jnp.broadcast_to(b1f[f:f + 1, :], (16, 128))
        w1s[D:D + 16, f * 128:(f + 1) * 128] = jnp.where(row16 < 2, bb, 0.0).astype(BF16)
    layernorm_tile(0)

    def down0(g, act, r0, r1):
        res = _dot(w2_tiles(range(A1))[r0:r1, :], act)
        for t in range(PGROUPS[g]):
            acc[PST[g] + t, r0:r1, :] = res[:, t * 128:(t + 1) * 128]

    prev = None
    for g in range(NP):
        tiles = [j for j in range(PST[g], PST[g] + PGROUPS[g]) if j >= 1]
        if g == 0:
            w1_cp(0, A1, S_X).wait()
        if g == 1:
            for f in range(A1):
                w2_cp(f, S_X + 1).wait()
        for j in tiles:
            x_cp(j).wait()
        if g == 0:
            w1T = w1s[:, 0:A1 * 128].T
        if prev is not None:
            down0(g - 1, prev, 0, DS[g - 1])
        for j in tiles:
            layernorm_tile(j)
        cur = ffn_up(w1T, PST[g], PGROUPS[g])
        if prev is not None:
            down0(g - 1, prev, DS[g - 1], D)
        prev = cur
    for cp in chunk_cps(FB, 1, S_B):
        cp.wait()
    w1Tb = w1s[:, FB * 128:(FB + 1) * 128].T
    for k in range(KT):
        w1Tbs[k] = pltpu.bitcast(w1Tb[:, k * 128:(k + 1) * 128], U32)
    down0(NP - 1, prev, 0, RBS[0])
    actb = ffn_up(w1Tb, 0, NBP)
    down0(NP - 1, prev, RBS[0], RBS[1])
    for cp in wq_cps():
        cp.wait()
    down0(NP - 1, prev, RBS[1], D)
    for k in range(KT):
        wqT[k] = pltpu.bitcast(wqs[k * 128:(k + 1) * 128, :].T, U32)
    for k in range(KT):
        woT[k] = pltpu.bitcast(wos[k * 128:(k + 1) * 128, :].T, U32)
    res = _dot(w2_tiles([FB]), actb)
    for t in range(NBP):
        acc[t] += res[:, t * 128:(t + 1) * 128]

    lane = jax.lax.broadcasted_iota(jnp.int32, (8, 128), 1)
    qk_scale = (DH ** -0.5) * LN2
    neg = -1e9 * LOG2E

    def windows(base, j, jp, r):
        cur = [qkv[j, pl.ds(base + r + u, 8, stride=DH), :] for u in range(2)]
        prv = [qkv[jp, pl.ds(base + r + u, 8, stride=DH), :] for u in range(2)]
        yield 0, cur
        for w in range(1, W):
            dl = DIL * w
            yield w, [pltpu.roll(jnp.where(lane >= 128 - dl, prv[u], cur[u]), dl, 1) for u in range(2)]

    def attention_tile(j):
        jp = jnp.maximum(j - 1, 0)
        pos = lane + j * 128
        for g in range(H // 8):
            lg = [None] * W
            for d in range(0, DH, 2):
                r = 8 * DH * g + d
                q = [qkv[j, pl.ds(r + u, 8, stride=DH), :] for u in range(2)]
                for w, ks in windows(D, j, jp, r):
                    t = q[0] * ks[0] + q[1] * ks[1]
                    lg[w] = t if d == 0 else lg[w] + t
                if (d // 2) % FQ == FQ - 1:
                    qkv[NT, 0:8, :] = lg[W - 1]
            lg = [lg[w] * qk_scale for w in range(W)]
            lg = [lg[0]] + [jnp.where(pos >= DIL * w, lg[w], neg) for w in range(1, W)]
            mx = functools.reduce(jnp.maximum, lg)
            p = [jnp.exp2(l - mx) for l in lg]
            rs = pl.reciprocal(functools.reduce(jnp.add, p), approx=True)
            p = [pw * rs for pw in p]
            pend = []
            for d in range(0, DH, 2):
                r = 8 * DH * g + d
                o = None
                for w, vs in windows(2 * D, j, jp, r):
                    t = [p[w] * vs[u] for u in range(2)]
                    o = t if o is None else [o[u] + t[u] for u in range(2)]
                pend += [(r + u, o[u]) for u in range(2)]
                if (d // 2) % FV == FV - 1 or d == DH - 2:
                    for rr, oo in pend:
                        qkv[j, pl.ds(rr, 8, stride=DH), :] = oo
                    pend = []

    def body(i, carry):
        @pl.when(i == 1)
        def _():
            for cp in rest_cps():
                cp.wait()

        f0 = FL + i * B
        c0 = pl.multiple_of(f0 * 128, 128)
        j0 = i * GT
        wq_all = jnp.concatenate([_as_bf16(wqT[k]) for k in range(KT)], axis=1)
        qkv_g = _dot(wq_all, xn_cols(j0, GT))
        for t in range(GT):
            qkv[j0 + t] = qkv_g[:, t * 128:(t + 1) * 128]
        w1T = w1s[:, pl.ds(c0, B * 128)].T
        act = ffn_up(w1T, 0, NT)
        for t in range(GT):
            attention_tile(j0 + t)
        res = _dot(w2_tiles([f0 + t for t in range(B)]), act)
        for t in range(NT):
            acc[t] += res[:, t * 128:(t + 1) * 128]
        wo_all = jnp.concatenate([_as_bf16(woT[k]) for k in range(KT)], axis=1)[:, 0:D]
        o_g = jnp.concatenate([qkv[j0 + t, 0:D, :] for t in range(GT)], axis=1).astype(BF16)
        res2 = _dot(wo_all, o_g)
        for t in range(GT):
            acc[j0 + t] += res2[:, t * 128:(t + 1) * 128]
        return carry

    for cp in chunk_cps(FL, B, S_L0):
        cp.wait()
    jax.lax.fori_loop(0, NL, body, 0)

    w1Te = w1s[:, FE * 128:].T
    w2e = w2_tiles([FE])
    w1Tb = jnp.concatenate([_as_bf16(w1Tbs[k]) for k in range(KT)], axis=1)
    w2e2 = w2_tiles([FB, FE])
    pre = {j: ffn_up(w1Tb, j, 1) for j in range(NBP, NBP + EPRE)}

    def up_e(j):
        a = ffn_up(w1Te, j, 1)
        if j >= NBP:
            ab = pre[j] if j in pre else ffn_up(w1Tb, j, 1)
            a = jnp.concatenate([ab, a], axis=0)
        return a

    nxt = up_e(0)
    for j in range(NT):
        act = nxt
        if j + 1 < NT:
            nxt = up_e(j + 1)
        w2c = w2e2 if j >= NBP else w2e
        for r0, r1 in out_parts(j):
            res = _dot(w2c[r0:r1, :], act)
            y = (acc[j, r0:r1, :] + res) * LN2 + xs[j, r0:r1, :].astype(F32)
            stg[j, r0:r1, :] = y.astype(BF16)
            out_cp(j, r0, r1).start()
    for j in range(NT):
        for r0, r1 in out_parts(j):
            out_cp(j, r0, r1).wait()


_SCRATCH = [
    pltpu.VMEM((NT, D, 128), BF16),
    pltpu.VMEM((NT, KP, 128), BF16),
    pltpu.VMEM((KP, F), BF16),
    pltpu.VMEM((NF, D, 128), BF16),
    pltpu.VMEM((KP, 3 * D), BF16),
    pltpu.VMEM((KT, 3 * D // 2, 128), U32),
    pltpu.VMEM((KP, D), BF16),
    pltpu.VMEM((KT, D // 2, 128), U32),
    pltpu.VMEM((NF, 128), BF16),
    pltpu.VMEM((NT, D, 128), F32),
    pltpu.VMEM((NT + 1, 3 * D, 128), F32),
    pltpu.VMEM((NT, D, 128), BF16),
    pltpu.VMEM((KT, 64, 128), U32),
    pltpu.SemaphoreType.DMA((NSEM,)),
]


@jax.jit
def pallas_parallel_sum__sliding_local_dilated__dense_activation_mish__prompt_kernel(
    A_x: jax.Array,
    A_wqkv: jax.Array,
    A_wo: jax.Array,
    B_x: jax.Array,
    B_w1: jax.Array,
    B_b1: jax.Array,
    B_w2: jax.Array,
):
    del B_x
    xt = jnp.transpose(A_x[0])
    w2t = jnp.transpose(B_w2)
    b1 = B_b1.reshape(NF, 128)
    out_t = pl.pallas_call(
        _kernel,
        in_specs=[pl.BlockSpec(memory_space=pl.ANY)] * 6,
        out_specs=pl.BlockSpec(memory_space=pl.ANY),
        out_shape=jax.ShapeDtypeStruct((D, S), BF16),
        scratch_shapes=_SCRATCH,
        compiler_params=pltpu.CompilerParams(vmem_limit_bytes=110 * 1024 * 1024),
        name="fused_block",
    )(xt, A_wqkv, A_wo, B_w1, b1, w2t)
    return jnp.transpose(out_t)[None]
```

```python
import functools

import jax
import jax.numpy as jnp
import jax.experimental.pallas as pl
import jax.experimental.pallas.tpu as pltpu

S, D, F = 2048, 576, 4608
H, DH, W, DIL = 32, 18, 8, 2
KP = 640
NT = S // 128
NF = F // 128
KT = KP // 128
LOG2E = 1.4426950408889634
LN2 = 0.6931471805599453
LOG2E_HI = 1.4453125
LOG2E_LO = LOG2E - LOG2E_HI
EPS = 1e-5
F32 = jnp.float32
BF16 = jnp.bfloat16
U32 = jnp.uint32

A1 = 2
FB = A1
FL = A1 + 1
FE = NF - 1
B = 4
GT = 2
NL = NT // GT
NBP = 12
EPRE = 2
PGROUPS = (2, 2, 4, 8)
NP = len(PGROUPS)
PST = [sum(PGROUPS[:g]) for g in range(NP)]
DS = (432, 432, 576, 480)
LASTN, LASTK = 6, 4
FQ = 2
FV = 2
assert FL + NL * B == FE and sum(PGROUPS) == NT

S_X0 = 0
S_X = 1
S_WQ = S_X + NP
S_L0 = S_WQ + 1
S_REST = S_L0 + 1
S_OUT = S_REST + 1
NSEM = S_OUT + 1


def _x_sem(j):
    return S_X0 if j == 0 else S_X + max(g for g in range(NP) if PST[g] <= j)


def _dot(a, b):
    return jnp.dot(a, b, preferred_element_type=F32)


def _as_bf16(u):
    return pltpu.bitcast(u, BF16)


def _mish_scaled(hs):
    e = jnp.exp2(jnp.minimum(hs, 13.0))
    n = e * (e + 2.0)
    return (hs * n) * pl.reciprocal(n + 2.0, approx=True)


def _kernel(x_hbm, wqkv_hbm, wo_hbm, w1_hbm, b1_hbm, w2_hbm, out_hbm,
            xs, xn, w1s, w2s, wqs, wqT, wos, woT, b1s, acc, qkv, stg, w1Tbs, sems):

    def x_cp(j):
        return pltpu.make_async_copy(x_hbm.at[:, j * 128:(j + 1) * 128], xs.at[j], sems.at[_x_sem(j)])

    def w1_cp(f0, nf, sem):
        cols = pl.ds(f0 * 128, nf * 128)
        return pltpu.make_async_copy(w1_hbm.at[:, cols], w1s.at[0:D, cols], sems.at[sem])

    def w2_cp(f, sem):
        return pltpu.make_async_copy(w2_hbm.at[:, pl.ds(f * 128, 128)], w2s.at[f], sems.at[sem])

    def chunk_cps(f0, nf, sem):
        return [w1_cp(f0, nf, sem)] + [w2_cp(f, sem) for f in range(f0, f0 + nf)]

    def b1_cp():
        return pltpu.make_async_copy(b1_hbm, b1s, sems.at[S_X0])

    def wq_cps():
        return [pltpu.make_async_copy(wqkv_hbm, wqs.at[0:D, :], sems.at[S_WQ]),
                pltpu.make_async_copy(wo_hbm, wos.at[0:D, :], sems.at[S_WQ])]

    def rest_cps():
        return chunk_cps(FL + B, NF - FL - B, S_REST)

    def out_cp(j, r0, r1):
        return pltpu.make_async_copy(stg.at[j, r0:r1, :], out_hbm.at[r0:r1, j * 128:(j + 1) * 128],
                                     sems.at[S_OUT])

    def out_parts(j):
        n = LASTN if j >= NT - LASTK else 1
        return [(q * D // n, (q + 1) * D // n) for q in range(n)]

    b1_cp().start()
    x_cp(0).start()
    w1_cp(0, A1, S_X).start()
    for j in range(1, PGROUPS[0]):
        x_cp(j).start()
    for f in range(A1):
        w2_cp(f, S_X + 1).start()
    for j in range(PGROUPS[0], NT):
        x_cp(j).start()
    for cp in chunk_cps(FB, 1, S_WQ) + wq_cps() + chunk_cps(FL, B, S_L0) + rest_cps():
        cp.start()

    def layernorm_tile(j):
        x = xs[j].astype(F32)
        m = jnp.sum(x, axis=0, keepdims=True) * (1.0 / D)
        xc = x - m
        v = jnp.sum(xc * xc, axis=0, keepdims=True) * (1.0 / D)
        r = jax.lax.rsqrt(v + EPS) * LOG2E
        xn[j, 0:D, :] = (xc * r).astype(BF16)

    def xn_cols(j0, n):
        return jnp.concatenate([xn[j0 + t] for t in range(n)], axis=1)

    def w2_tiles(fs):
        return jnp.concatenate([w2s[f] for f in fs], axis=1)

    def ffn_up(w1T, j0, n):
        return _mish_scaled(_dot(w1T, xn_cols(j0, n))).astype(BF16)

    w1s[D + 16:KP, :] = jnp.zeros((KP - D - 16, F), BF16)
    wqs[D:KP, :] = jnp.zeros((KP - D, 3 * D), BF16)
    wos[D:KP, :] = jnp.zeros((KP - D, D), BF16)
    row = jax.lax.broadcasted_iota(jnp.int32, (KP - D, 128), 0)
    ones_rows = jnp.where(row == 0, LOG2E_HI, jnp.where(row == 1, LOG2E_LO, 0.0)).astype(BF16)
    for j in range(NT):
        xn[j, D:KP, :] = ones_rows
    b1_cp().wait()
    x_cp(0).wait()
    b1f = b1s[...].astype(F32)
    row16 = jax.lax.broadcasted_iota(jnp.int32, (16, 128), 0)
    for f in range(NF):
        bb = jnp.broadcast_to(b1f[f:f + 1, :], (16, 128))
        w1s[D:D + 16, f * 128:(f + 1) * 128] = jnp.where(row16 < 2, bb, 0.0).astype(BF16)
    layernorm_tile(0)

    def down0(g, act, r0, r1):
        if r0 == r1:
            return
        res = _dot(w2_tiles(range(A1))[r0:r1, :], act)
        for t in range(PGROUPS[g]):
            acc[PST[g] + t, r0:r1, :] = res[:, t * 128:(t + 1) * 128]

    prev = None
    for g in range(NP):
        tiles = [j for j in range(PST[g], PST[g] + PGROUPS[g]) if j >= 1]
        if g == 0:
            w1_cp(0, A1, S_X).wait()
        if g == 1:
            for f in range(A1):
                w2_cp(f, S_X + 1).wait()
        for j in tiles:
            x_cp(j).wait()
        if g == 0:
            w1T = w1s[:, 0:A1 * 128].T
        if prev is not None:
            down0(g - 1, prev, 0, DS[g - 1])
        for j in tiles:
            layernorm_tile(j)
        if PGROUPS[g] % 4:
            cur = jnp.concatenate([ffn_up(w1T[0:128, :], PST[g], PGROUPS[g]),
                                   ffn_up(w1T[128:256, :], PST[g], PGROUPS[g])], axis=0)
        else:
            cur = ffn_up(w1T, PST[g], PGROUPS[g])
        if prev is not None:
            down0(g - 1, prev, DS[g - 1], D)
        prev = cur
    down0(NP - 1, prev, 0, DS[NP - 1])
    for cp in chunk_cps(FB, 1, S_WQ) + wq_cps():
        cp.wait()
    w1Tb = w1s[:, FB * 128:(FB + 1) * 128].T
    for k in range(KT):
        w1Tbs[k] = pltpu.bitcast(w1Tb[:, k * 128:(k + 1) * 128], U32)
    down0(NP - 1, prev, DS[NP - 1], D)
    actb = ffn_up(w1Tb, 0, NBP)
    for k in range(KT):
        wqT[k] = pltpu.bitcast(wqs[k * 128:(k + 1) * 128, :].T, U32)
    for k in range(KT):
        woT[k] = pltpu.bitcast(wos[k * 128:(k + 1) * 128, :].T, U32)
    res = _dot(w2_tiles([FB]), actb)
    for t in range(NBP):
        acc[t] += res[:, t * 128:(t + 1) * 128]

    lane = jax.lax.broadcasted_iota(jnp.int32, (8, 128), 1)
    qk_scale = (DH ** -0.5) * LN2
    neg = -1e9 * LOG2E

    def windows(base, j, jp, r):
        cur = [qkv[j, pl.ds(base + r + u, 8, stride=DH), :] for u in range(2)]
        prv = [qkv[jp, pl.ds(base + r + u, 8, stride=DH), :] for u in range(2)]
        yield 0, cur
        for w in range(1, W):
            dl = DIL * w
            yield w, [pltpu.roll(jnp.where(lane >= 128 - dl, prv[u], cur[u]), dl, 1) for u in range(2)]

    def attention_tile(j):
        jp = jnp.maximum(j - 1, 0)
        pos = lane + j * 128
        for g in range(H // 8):
            lg = [None] * W
            for d in range(0, DH, 2):
                r = 8 * DH * g + d
                q = [qkv[j, pl.ds(r + u, 8, stride=DH), :] for u in range(2)]
                for w, ks in windows(D, j, jp, r):
                    t = q[0] * ks[0] + q[1] * ks[1]
                    lg[w] = t if d == 0 else lg[w] + t
                if (d // 2) % FQ == FQ - 1:
                    qkv[NT, 0:8, :] = lg[W - 1]
            lg = [lg[w] * qk_scale for w in range(W)]
            lg = [lg[0]] + [jnp.where(pos >= DIL * w, lg[w], neg) for w in range(1, W)]
            mx = functools.reduce(jnp.maximum, lg)
            p = [jnp.exp2(l - mx) for l in lg]
            rs = pl.reciprocal(functools.reduce(jnp.add, p), approx=True)
            p = [pw * rs for pw in p]
            pend = []
            for d in range(0, DH, 2):
                r = 8 * DH * g + d
                o = None
                for w, vs in windows(2 * D, j, jp, r):
                    t = [p[w] * vs[u] for u in range(2)]
                    o = t if o is None else [o[u] + t[u] for u in range(2)]
                pend += [(r + u, o[u]) for u in range(2)]
                if (d // 2) % FV == FV - 1 or d == DH - 2:
                    for rr, oo in pend:
                        qkv[j, pl.ds(rr, 8, stride=DH), :] = oo
                    pend = []

    def body(i, carry):
        @pl.when(i == 1)
        def _():
            for cp in rest_cps():
                cp.wait()

        f0 = FL + i * B
        c0 = pl.multiple_of(f0 * 128, 128)
        j0 = i * GT
        wq_all = jnp.concatenate([_as_bf16(wqT[k]) for k in range(KT)], axis=1)
        qkv_g = _dot(wq_all, xn_cols(j0, GT))
        for t in range(GT):
            qkv[j0 + t] = qkv_g[:, t * 128:(t + 1) * 128]
        w1T = w1s[:, pl.ds(c0, B * 128)].T
        act = ffn_up(w1T, 0, NT)
        for t in range(GT):
            attention_tile(j0 + t)
        res = _dot(w2_tiles([f0 + t for t in range(B)]), act)
        for t in range(NT):
            acc[t] += res[:, t * 128:(t + 1) * 128]
        wo_all = jnp.concatenate([_as_bf16(woT[k]) for k in range(KT)], axis=1)[:, 0:D]
        o_g = jnp.concatenate([qkv[j0 + t, 0:D, :] for t in range(GT)], axis=1).astype(BF16)
        res2 = _dot(wo_all, o_g)
        for t in range(GT):
            acc[j0 + t] += res2[:, t * 128:(t + 1) * 128]
        return carry

    for cp in chunk_cps(FL, B, S_L0):
        cp.wait()
    jax.lax.fori_loop(0, NL, body, 0)

    w1Te = w1s[:, FE * 128:].T
    w2e = w2_tiles([FE])
    w1Tb = jnp.concatenate([_as_bf16(w1Tbs[k]) for k in range(KT)], axis=1)
    w2e2 = w2_tiles([FB, FE])
    pre = {j: ffn_up(w1Tb, j, 1) for j in range(NBP, NBP + EPRE)}

    def up_e(j):
        a = ffn_up(w1Te, j, 1)
        if j >= NBP:
            ab = pre[j] if j in pre else ffn_up(w1Tb, j, 1)
            a = jnp.concatenate([ab, a], axis=0)
        return a

    nxt = up_e(0)
    for j in range(NT):
        act = nxt
        if j + 1 < NT:
            nxt = up_e(j + 1)
        w2c = w2e2 if j >= NBP else w2e
        for r0, r1 in out_parts(j):
            res = _dot(w2c[r0:r1, :], act)
            y = (acc[j, r0:r1, :] + res) * LN2 + xs[j, r0:r1, :].astype(F32)
            stg[j, r0:r1, :] = y.astype(BF16)
            out_cp(j, r0, r1).start()
    for j in range(NT):
        for r0, r1 in out_parts(j):
            out_cp(j, r0, r1).wait()


_SCRATCH = [
    pltpu.VMEM((NT, D, 128), BF16),
    pltpu.VMEM((NT, KP, 128), BF16),
    pltpu.VMEM((KP, F), BF16),
    pltpu.VMEM((NF, D, 128), BF16),
    pltpu.VMEM((KP, 3 * D), BF16),
    pltpu.VMEM((KT, 3 * D // 2, 128), U32),
    pltpu.VMEM((KP, D), BF16),
    pltpu.VMEM((KT, D // 2, 128), U32),
    pltpu.VMEM((NF, 128), BF16),
    pltpu.VMEM((NT, D, 128), F32),
    pltpu.VMEM((NT + 1, 3 * D, 128), F32),
    pltpu.VMEM((NT, D, 128), BF16),
    pltpu.VMEM((KT, 64, 128), U32),
    pltpu.SemaphoreType.DMA((NSEM,)),
]


@jax.jit
def pallas_parallel_sum__sliding_local_dilated__dense_activation_mish__prompt_kernel(
    A_x: jax.Array,
    A_wqkv: jax.Array,
    A_wo: jax.Array,
    B_x: jax.Array,
    B_w1: jax.Array,
    B_b1: jax.Array,
    B_w2: jax.Array,
):
    del B_x
    xt = jnp.transpose(A_x[0])
    w2t = jnp.transpose(B_w2)
    b1 = B_b1.reshape(NF, 128)
    out_t = pl.pallas_call(
        _kernel,
        in_specs=[pl.BlockSpec(memory_space=pl.ANY)] * 6,
        out_specs=pl.BlockSpec(memory_space=pl.ANY),
        out_shape=jax.ShapeDtypeStruct((D, S), BF16),
        scratch_shapes=_SCRATCH,
        compiler_params=pltpu.CompilerParams(vmem_limit_bytes=110 * 1024 * 1024),
        name="fused_block",
    )(xt, A_wqkv, A_wo, B_w1, b1, w2t)
    return jnp.transpose(out_t)[None]
```
